```python
import os as _os
_os.environ.setdefault("JAX_PLATFORMS", "cpu")
import jax
import jax.numpy as jnp

def _softmax(x, axis=-1):
    return jax.nn.softmax(x, axis=axis)
def _gelu(x):
    return jax.nn.gelu(x, approximate=True)
def _silu(x):
    return jax.nn.silu(x)
def _sigmoid(x):
    return jax.nn.sigmoid(x)
def _layernorm(x, axis=-1, eps=1e-5):
    m = jnp.mean(x, axis=axis, keepdims=True)
    v = jnp.var(x, axis=axis, keepdims=True)
    return (x - m) / jnp.sqrt(v + eps)
def _scatter_add(tgt, idx, src, axis=0):
    return tgt.at[idx].add(src)
def _segment_sum(src, seg, n):
    return jax.ops.segment_sum(src, seg, n)
class _Rng:
    def __init__(self, key):
        self._k = key
    def _next(self):
        self._k, sub = jax.random.split(self._k)
        return sub
    def normal(self, shape):
        return jax.random.normal(self._next(), shape, dtype=jnp.bfloat16)
    def randint(self, lo, hi, shape):
        return jax.random.randint(self._next(), shape, lo, hi, dtype=jnp.int32)
    def uniform(self, shape, lo=0.0, hi=1.0):
        return jax.random.uniform(self._next(), shape, jnp.bfloat16, lo, hi)
    def permutation(self, n):
        return jax.random.permutation(self._next(), n)


kernel_name = 'parallel_sum__ssm_conv_s5__geglu_ffn__prompt'

def setup_inputs():
    _rng = _Rng(jax.random.key(int.from_bytes(__import__("os").urandom(4), "little")))
    _w = (lambda a: (lambda t: t.astype(jnp.bfloat16) if jnp.issubdtype(t.dtype, jnp.floating) else t)(jnp.asarray(a)))
    def _A_setup():
        B, S, D = 1, 2048, 512
        P = D
        Lambda_re = -0.5 * jnp.exp((lambda *s: _rng.normal(s) * 0.8)(P))
        Lambda_im = (lambda *s: _rng.normal(s) * 0.8)(P) * 1.0
        B_re = (lambda *s: _rng.normal(s) * 0.8)(P, D) * (D ** -0.5)
        B_im = (lambda *s: _rng.normal(s) * 0.8)(P, D) * (D ** -0.5)
        C_re = (lambda *s: _rng.normal(s) * 0.8)(D, P) * (P ** -0.5)
        C_im = (lambda *s: _rng.normal(s) * 0.8)(D, P) * (P ** -0.5)
        log_dt = (lambda *s: _rng.normal(s) * 0.8)(P) * 0.3 - 2.0
        Dskip = (lambda *s: _rng.normal(s) * 0.8)(D)
        return {
            "x": _w((lambda *s: _rng.normal(s) * 0.05)(B, S, D)),
            "Lambda_re": _w(Lambda_re),
            "Lambda_im": _w(Lambda_im),
            "B_re": _w(B_re),
            "B_im": _w(B_im),
            "C_re": _w(C_re),
            "C_im": _w(C_im),
            "log_dt": _w(log_dt),
            "Dskip": _w(Dskip),
        }
    _A_in = _A_setup()

    def _B_setup():
        B, S, D, F = 1, 2048, 512, 1376
        return {
            "x": _w((lambda *s: _rng.normal(s) * 0.05)(B, S, D)),
            "w_gate": _w((lambda *s: _rng.normal(s) * 0.05)(D, F)),
            "w_up": _w((lambda *s: _rng.normal(s) * 0.05)(D, F)),
            "w_down": _w((lambda *s: _rng.normal(s) * 0.05)(F, D)),
        }
    _B_in = _B_setup()

    return {
        "A_x": _A_in["x"],
        "A_Lambda_re": _A_in["Lambda_re"],
        "A_Lambda_im": _A_in["Lambda_im"],
        "A_B_re": _A_in["B_re"],
        "A_B_im": _A_in["B_im"],
        "A_C_re": _A_in["C_re"],
        "A_C_im": _A_in["C_im"],
        "A_log_dt": _A_in["log_dt"],
        "A_Dskip": _A_in["Dskip"],
        "B_x": _B_in["x"],
        "B_w_gate": _B_in["w_gate"],
        "B_w_up": _B_in["w_up"],
        "B_w_down": _B_in["w_down"],
    }

def reference(A_x, A_Lambda_re, A_Lambda_im, A_B_re, A_B_im, A_C_re, A_C_im, A_log_dt, A_Dskip, B_x, B_w_gate, B_w_up, B_w_down):
    def _A_ref(x, Lambda_re, Lambda_im, B_re, B_im, C_re, C_im, log_dt, Dskip):
        Bsz, L, H = x.shape
        Lam = Lambda_re + 1j * Lambda_im
        Bmat = B_re + 1j * B_im
        Cmat = C_re + 1j * C_im
        dt = jnp.exp(log_dt)
        Lam_bar = jnp.exp(dt * Lam)
        B_bar = ((Lam_bar - 1.0) / Lam)[:, None] * Bmat
        Bu = jnp.einsum("bld,pd->blp", x + 0j, B_bar)
        h = jnp.zeros_like(Bu[:, 0, :])
        hs = []
        for t in range(L):
            h = Lam_bar[None, :] * h + Bu[:, t, :]
            hs.append(h)
        hseq = jnp.stack(hs, 1)
        y = 2.0 * jnp.einsum("blp,dp->bld", hseq, Cmat).real + x * Dskip[None, None, :]
        return y

    def _B_ref(x, w_gate, w_up, w_down):
        return (_gelu(x @ w_gate) * (x @ w_up)) @ w_down

    x = A_x
    xn = _layernorm(x, axis=-1)
    return x + _A_ref(xn, A_Lambda_re, A_Lambda_im, A_B_re, A_B_im, A_C_re, A_C_im, A_log_dt, A_Dskip) + _B_ref(xn, B_w_gate, B_w_up, B_w_down)
```

```python
import functools

import jax
import jax.numpy as jnp
import jax.experimental.pallas as pl
import jax.experimental.pallas.tpu as pltpu

_NT = (((1,), (1,)), ((), ()))


def _kernel(x_ref, lre_ref, lim_ref, ldt_ref, dsk_ref, bre_ref, bim_ref,
            cre_ref, cim_ref, wg_ref, wu_ref, wd_ref, o_ref,
            cw_ref, par_ref, st_ref, bu_ref, hs_ref, *, T, P):
    S = T // 8
    f32 = jnp.float32
    bf16 = jnp.bfloat16

    @pl.when(pl.program_id(0) == 0)
    def _init():
        lre = lre_ref[...].astype(f32)
        lim = lim_ref[...].astype(f32)
        dt = jnp.exp(ldt_ref[...].astype(f32)).astype(bf16).astype(f32)
        mag = jnp.exp(dt * lre)
        ang = dt * lim
        a = mag * jnp.cos(ang)
        b = mag * jnp.sin(ang)
        den = lre * lre + lim * lim
        xr = a - 1.0
        cr = (xr * lre + b * lim) / den
        ci = (b * lre - xr * lim) / den
        cre = cre_ref[...].astype(f32)
        cim = cim_ref[...].astype(f32)
        cw_ref[:, 0:P] = (2.0 * (cre * cr - cim * ci)).astype(bf16)
        cw_ref[:, P:2 * P] = (-2.0 * (cre * ci + cim * cr)).astype(bf16)
        aS, bS = a, b
        n = 1
        while n < S:
            aS, bS = aS * aS - bS * bS, 2.0 * aS * bS
            n *= 2
        par_ref[0:1, :] = a
        par_ref[1:2, :] = b
        par_ref[2:3, :] = aS
        par_ref[3:4, :] = bS
        par_ref[4:8, :] = jnp.zeros((4, P), f32)
        st_ref[...] = jnp.zeros(st_ref.shape, f32)

    x = x_ref[...].astype(f32)
    m = jnp.mean(x, axis=-1, keepdims=True)
    xc = x - m
    v = jnp.mean(xc * xc, axis=-1, keepdims=True)
    xn = xc * jax.lax.rsqrt(v + 1e-5)
    xnb = xn.astype(bf16)

    G = P // 128
    bur = jax.lax.dot_general(xnb, bre_ref[...], _NT, preferred_element_type=f32)
    bui = jax.lax.dot_general(xnb, bim_ref[...], _NT, preferred_element_type=f32)
    for g in range(G):
        bu_ref[g] = bur[:, g * 128:(g + 1) * 128]
        bu_ref[G + g] = bui[:, g * 128:(g + 1) * 128]

    def ld(j, off):
        return jnp.concatenate(
            [bu_ref[off + g, pl.ds(j, 8, stride=S), :] for g in range(G)], axis=1)

    a8 = jnp.broadcast_to(par_ref[0:1, :], (8, P))
    b8 = jnp.broadcast_to(par_ref[1:2, :], (8, P))

    hr = jnp.zeros((8, P), f32)
    hi = jnp.zeros((8, P), f32)
    for j in range(S):
        br = ld(j, 0)
        bi = ld(j, G)
        hr, hi = a8 * hr - b8 * hi + br, a8 * hi + b8 * hr + bi

    aS = par_ref[2:3, :]
    bS = par_ref[3:4, :]
    cr_ = st_ref[0:1, :]
    ci_ = st_ref[1:2, :]
    rows_r, rows_i = [], []
    for c in range(8):
        rows_r.append(cr_)
        rows_i.append(ci_)
        cr_, ci_ = (aS * cr_ - bS * ci_ + hr[c:c + 1, :], aS * ci_ + bS * cr_ + hi[c:c + 1, :])
    st_ref[0:1, :] = cr_
    st_ref[1:2, :] = ci_
    hr = jnp.concatenate(rows_r, axis=0)
    hi = jnp.concatenate(rows_i, axis=0)

    for j in range(S):
        br = ld(j, 0)
        bi = ld(j, G)
        hr, hi = a8 * hr - b8 * hi + br, a8 * hi + b8 * hr + bi
        for g in range(G):
            hs_ref[g, pl.ds(j, 8, stride=S), :] = hr[:, g * 128:(g + 1) * 128]
            hs_ref[G + g, pl.ds(j, 8, stride=S), :] = hi[:, g * 128:(g + 1) * 128]

    hs = jnp.concatenate([hs_ref[g].astype(bf16) for g in range(2 * G)], axis=1)
    y = jax.lax.dot_general(hs, cw_ref[...], _NT, preferred_element_type=f32)

    g = jnp.dot(xnb, wg_ref[...], preferred_element_type=f32)
    u = jnp.dot(xnb, wu_ref[...], preferred_element_type=f32)
    act = (jax.nn.gelu(g, approximate=True) * u).astype(bf16)
    ffn = jnp.dot(act, wd_ref[...], preferred_element_type=f32)

    o_ref[...] = x + y + xn * dsk_ref[...].astype(f32) + ffn


@jax.jit
def pallas_parallel_sum__ssm_conv_s5__geglu_ffn__prompt_kernel(
    A_x: jax.Array,
    A_Lambda_re: jax.Array,
    A_Lambda_im: jax.Array,
    A_B_re: jax.Array,
    A_B_im: jax.Array,
    A_C_re: jax.Array,
    A_C_im: jax.Array,
    A_log_dt: jax.Array,
    A_Dskip: jax.Array,
    B_x: jax.Array,
    B_w_gate: jax.Array,
    B_w_up: jax.Array,
    B_w_down: jax.Array,
):
    Bsz, L, D = A_x.shape
    assert Bsz == 1
    P = A_Lambda_re.shape[0]
    F = B_w_gate.shape[1]
    T = 256
    x2 = A_x.reshape(L, D)
    row = lambda v: v.reshape(1, -1)

    const = lambda shape: pl.BlockSpec(shape, lambda i: (0, 0))
    out = pl.pallas_call(
        functools.partial(_kernel, T=T, P=P),
        grid=(L // T,),
        in_specs=[
            pl.BlockSpec((T, D), lambda i: (i, 0)),
            const((1, P)), const((1, P)), const((1, P)), const((1, D)),
            const((P, D)), const((P, D)), const((D, P)), const((D, P)),
            const((D, F)), const((D, F)), const((F, D)),
        ],
        out_specs=pl.BlockSpec((T, D), lambda i: (i, 0)),
        out_shape=jax.ShapeDtypeStruct((L, D), jnp.float32),
        scratch_shapes=[
            pltpu.VMEM((D, 2 * P), jnp.bfloat16),
            pltpu.VMEM((8, P), jnp.float32),
            pltpu.VMEM((8, P), jnp.float32),
            pltpu.VMEM((2 * P // 128, T, 128), jnp.float32),
            pltpu.VMEM((2 * P // 128, T, 128), jnp.float32),
        ],
        compiler_params=pltpu.CompilerParams(
            dimension_semantics=("arbitrary",),
            vmem_limit_bytes=100 * 1024 * 1024,
        ),
    )(x2, row(A_Lambda_re), row(A_Lambda_im), row(A_log_dt), row(A_Dskip),
      A_B_re, A_B_im, A_C_re, A_C_im, B_w_gate, B_w_up, B_w_down)
    return out.reshape(Bsz, L, D)
```

```python
import functools

import jax
import jax.numpy as jnp
import jax.experimental.pallas as pl
import jax.experimental.pallas.tpu as pltpu

_NT = (((1,), (1,)), ((), ()))


def _kernel(x_ref, lre_ref, lim_ref, ldt_ref, dsk_ref, bre_ref, bim_ref,
            cre_ref, cim_ref, wg_ref, wu_ref, wd_ref, o_ref,
            cw_ref, par_ref, st_ref, bu_ref, hs_ref, *, T, P):
    S = T // 8
    f32 = jnp.float32
    bf16 = jnp.bfloat16

    @pl.when(pl.program_id(0) == 0)
    def _init():
        lre = lre_ref[...].astype(f32)
        lim = lim_ref[...].astype(f32)
        dt = jnp.exp(ldt_ref[...].astype(f32)).astype(bf16).astype(f32)
        mag = jnp.exp(dt * lre)
        ang = dt * lim
        a = mag * jnp.cos(ang)
        b = mag * jnp.sin(ang)
        den = lre * lre + lim * lim
        xr = a - 1.0
        cr = (xr * lre + b * lim) / den
        ci = (b * lre - xr * lim) / den
        cre = cre_ref[...].astype(f32)
        cim = cim_ref[...].astype(f32)
        cw_ref[:, 0:P] = (2.0 * (cre * cr - cim * ci)).astype(bf16)
        cw_ref[:, P:2 * P] = (-2.0 * (cre * ci + cim * cr)).astype(bf16)
        aS, bS = a, b
        n = 1
        while n < S:
            aS, bS = aS * aS - bS * bS, 2.0 * aS * bS
            n *= 2
        par_ref[0:1, :] = a
        par_ref[1:2, :] = b
        par_ref[2:3, :] = aS
        par_ref[3:4, :] = bS
        par_ref[4:8, :] = jnp.zeros((4, P), f32)
        st_ref[...] = jnp.zeros(st_ref.shape, f32)

    x = x_ref[...].astype(f32)
    m = jnp.mean(x, axis=-1, keepdims=True)
    xc = x - m
    v = jnp.mean(xc * xc, axis=-1, keepdims=True)
    xn = xc * jax.lax.rsqrt(v + 1e-5)
    xnb = xn.astype(bf16)

    G = P // 128
    bur = jax.lax.dot_general(xnb, bre_ref[...], _NT, preferred_element_type=f32)
    bui = jax.lax.dot_general(xnb, bim_ref[...], _NT, preferred_element_type=f32)
    for g in range(G):
        bu_ref[g] = bur[:, g * 128:(g + 1) * 128]
        bu_ref[G + g] = bui[:, g * 128:(g + 1) * 128]

    def ld(j, off):
        return jnp.concatenate(
            [bu_ref[off + g, pl.ds(j, 8, stride=S), :] for g in range(G)], axis=1)

    a8 = jnp.broadcast_to(par_ref[0:1, :], (8, P))
    b8 = jnp.broadcast_to(par_ref[1:2, :], (8, P))

    hr = jnp.zeros((8, P), f32)
    hi = jnp.zeros((8, P), f32)
    for j in range(S):
        br = ld(j, 0)
        bi = ld(j, G)
        hr, hi = a8 * hr - b8 * hi + br, a8 * hi + b8 * hr + bi

    aS = par_ref[2:3, :]
    bS = par_ref[3:4, :]
    cr_ = st_ref[0:1, :]
    ci_ = st_ref[1:2, :]
    rows_r, rows_i = [], []
    for c in range(8):
        rows_r.append(cr_)
        rows_i.append(ci_)
        cr_, ci_ = (aS * cr_ - bS * ci_ + hr[c:c + 1, :], aS * ci_ + bS * cr_ + hi[c:c + 1, :])
    st_ref[0:1, :] = cr_
    st_ref[1:2, :] = ci_
    hr = jnp.concatenate(rows_r, axis=0)
    hi = jnp.concatenate(rows_i, axis=0)

    for j in range(S):
        br = ld(j, 0)
        bi = ld(j, G)
        hr, hi = a8 * hr - b8 * hi + br, a8 * hi + b8 * hr + bi
        for g in range(G):
            hs_ref[g, pl.ds(j, 8, stride=S), :] = hr[:, g * 128:(g + 1) * 128]
            hs_ref[G + g, pl.ds(j, 8, stride=S), :] = hi[:, g * 128:(g + 1) * 128]

    hs = jnp.concatenate([hs_ref[g].astype(bf16) for g in range(2 * G)], axis=1)
    y = jax.lax.dot_general(hs, cw_ref[...], _NT, preferred_element_type=f32)

    g = jax.lax.dot_general(xnb, wg_ref[...], _NT, preferred_element_type=f32)
    u = jax.lax.dot_general(xnb, wu_ref[...], _NT, preferred_element_type=f32)
    act = (jax.nn.gelu(g, approximate=True) * u).astype(bf16)
    ffn = jnp.dot(act, wd_ref[...], preferred_element_type=f32)

    o_ref[...] = x + y + xn * dsk_ref[...].astype(f32) + ffn


@jax.jit
def pallas_parallel_sum__ssm_conv_s5__geglu_ffn__prompt_kernel(
    A_x: jax.Array,
    A_Lambda_re: jax.Array,
    A_Lambda_im: jax.Array,
    A_B_re: jax.Array,
    A_B_im: jax.Array,
    A_C_re: jax.Array,
    A_C_im: jax.Array,
    A_log_dt: jax.Array,
    A_Dskip: jax.Array,
    B_x: jax.Array,
    B_w_gate: jax.Array,
    B_w_up: jax.Array,
    B_w_down: jax.Array,
):
    Bsz, L, D = A_x.shape
    assert Bsz == 1
    P = A_Lambda_re.shape[0]
    F = B_w_gate.shape[1]
    T = 256
    x2 = A_x.reshape(L, D)
    row = lambda v: v.reshape(1, -1)

    const = lambda shape: pl.BlockSpec(shape, lambda i: (0, 0))
    out = pl.pallas_call(
        functools.partial(_kernel, T=T, P=P),
        grid=(L // T,),
        in_specs=[
            pl.BlockSpec((T, D), lambda i: (i, 0)),
            const((1, P)), const((1, P)), const((1, P)), const((1, D)),
            const((P, D)), const((P, D)), const((D, P)), const((D, P)),
            const((F, D)), const((F, D)), const((F, D)),
        ],
        out_specs=pl.BlockSpec((T, D), lambda i: (i, 0)),
        out_shape=jax.ShapeDtypeStruct((L, D), jnp.float32),
        scratch_shapes=[
            pltpu.VMEM((D, 2 * P), jnp.bfloat16),
            pltpu.VMEM((8, P), jnp.float32),
            pltpu.VMEM((8, P), jnp.float32),
            pltpu.VMEM((2 * P // 128, T, 128), jnp.float32),
            pltpu.VMEM((2 * P // 128, T, 128), jnp.float32),
        ],
        compiler_params=pltpu.CompilerParams(
            dimension_semantics=("arbitrary",),
            vmem_limit_bytes=100 * 1024 * 1024,
        ),
    )(x2, row(A_Lambda_re), row(A_Lambda_im), row(A_log_dt), row(A_Dskip),
      A_B_re, A_B_im, A_C_re, A_C_im, B_w_gate.T, B_w_up.T, B_w_down)
    return out.reshape(Bsz, L, D)
```

```python
import functools

import jax
import jax.numpy as jnp
import jax.experimental.pallas as pl
import jax.experimental.pallas.tpu as pltpu

_NT = (((1,), (1,)), ((), ()))


def _kernel(x0_ref, xn_ref, lre_ref, lim_ref, ldt_ref, dsk_ref, bre_hbm, bim_hbm,
            cre_hbm, cim_hbm, wg_hbm, wu_hbm, wd_hbm, o_ref,
            bre_ref, bim_ref, cre_ref, cim_ref, wg_ref, wu_ref, wd_ref, sems,
            cw_ref, par_ref, st_ref, bu_ref, hs_ref, xb_ref, base_ref, *, T, P, F, FC, DG, NLN):
    S = T // 8
    SP = S + 1
    G = P // 128
    f32 = jnp.float32
    bf16 = jnp.bfloat16
    fchunks = [(k, min(k + FC, F)) for k in range(0, F, FC)]
    nfc = len(fchunks)
    dgroups = [(fchunks[k][0], fchunks[min(k + DG, nfc) - 1][1]) for k in range(0, nfc, DG)]

    cp_b = [pltpu.make_async_copy(bre_hbm, bre_ref, sems.at[0]),
            pltpu.make_async_copy(bim_hbm, bim_ref, sems.at[1])]
    cp_f = []
    for n, (f0, f1) in enumerate(dgroups):
        cp_f.append((
            pltpu.make_async_copy(wg_hbm.at[f0:f1, :], wg_ref.at[f0:f1, :], sems.at[5 + 2 * n]),
            pltpu.make_async_copy(wu_hbm.at[f0:f1, :], wu_ref.at[f0:f1, :], sems.at[6 + 2 * n])))
    cp_c = [pltpu.make_async_copy(cre_hbm, cre_ref, sems.at[2]),
            pltpu.make_async_copy(cim_hbm, cim_ref, sems.at[3])]
    cp_d = pltpu.make_async_copy(wd_hbm, wd_ref, sems.at[4])

    def layernorm(src_ref, slot, r0, r1):
        x = src_ref[r0:r1, :].astype(f32)
        m = jnp.mean(x, axis=-1, keepdims=True)
        xc = x - m
        v = jnp.mean(xc * xc, axis=-1, keepdims=True)
        xn = xc * jax.lax.rsqrt(v + 1e-5)
        xb_ref[slot, r0:r1, :] = xn.astype(bf16)
        base_ref[slot, r0:r1, :] = x + xn * dsk_ref[...].astype(f32).reshape(1, -1)

    cur = pl.program_id(0) % 2
    nxt = 1 - cur

    def body(first):
        if first:
            for c in cp_b:
                c.start()
            for cg, cu in cp_f:
                cg.start()
                cu.start()
            for c in cp_c:
                c.start()
            cp_d.start()
            lre = lre_ref[...].astype(f32).reshape(1, P)
            lim = lim_ref[...].astype(f32).reshape(1, P)
            dt = jnp.exp(ldt_ref[...].astype(f32).reshape(1, P)).astype(bf16).astype(f32)
            mag = jnp.exp(dt * lre)
            ang = dt * lim
            a = mag * jnp.cos(ang)
            b = mag * jnp.sin(ang)
            den = lre * lre + lim * lim
            xr = a - 1.0
            cr = (xr * lre + b * lim) / den
            ci = (b * lre - xr * lim) / den
            aS, bS = a, b
            n = 1
            while n < S:
                aS, bS = aS * aS - bS * bS, 2.0 * aS * bS
                n *= 2
            par_ref[0:1, :] = a
            par_ref[1:2, :] = b
            par_ref[2:3, :] = aS
            par_ref[3:4, :] = bS
            par_ref[4:8, :] = jnp.zeros((4, P), f32)
            st_ref[...] = jnp.zeros(st_ref.shape, f32)
            layernorm(x0_ref, 0, 0, T)
            for c in cp_b:
                c.wait()

        xnb = xb_ref[cur]
        bur = jax.lax.dot_general(xnb, bre_ref[...], _NT, preferred_element_type=f32)
        bui = jax.lax.dot_general(xnb, bim_ref[...], _NT, preferred_element_type=f32)
        for g in range(G):
            for c in range(8):
                bu_ref[g, c * SP:c * SP + S, :] = bur[c * S:(c + 1) * S, g * 128:(g + 1) * 128]
                bu_ref[G + g, c * SP:c * SP + S, :] = bui[c * S:(c + 1) * S, g * 128:(g + 1) * 128]

        def ld(j, off):
            return jnp.concatenate(
                [bu_ref[off + g, pl.ds(j, 8, stride=SP), :] for g in range(G)], axis=1)

        a8 = jnp.broadcast_to(par_ref[0:1, :], (8, P))
        b8 = jnp.broadcast_to(par_ref[1:2, :], (8, P))

        state = {}

        def pass1(j):
            hr, hi = state['h']
            br = ld(j, 0)
            bi = ld(j, G)
            state['h'] = (a8 * hr - b8 * hi + br, a8 * hi + b8 * hr + bi)

        def carry():
            hr, hi = state['h']
            aS = par_ref[2:3, :]
            bS = par_ref[3:4, :]
            cr_ = st_ref[0:1, :]
            ci_ = st_ref[1:2, :]
            rows_r, rows_i = [], []
            for c in range(8):
                rows_r.append(cr_)
                rows_i.append(ci_)
                cr_, ci_ = (aS * cr_ - bS * ci_ + hr[c:c + 1, :], aS * ci_ + bS * cr_ + hi[c:c + 1, :])
            st_ref[0:1, :] = cr_
            st_ref[1:2, :] = ci_
            state['h'] = (jnp.concatenate(rows_r, axis=0), jnp.concatenate(rows_i, axis=0))

        def pass2(j):
            hr, hi = state['h']
            br = ld(j, 0)
            bi = ld(j, G)
            hr, hi = a8 * hr - b8 * hi + br, a8 * hi + b8 * hr + bi
            state['h'] = (hr, hi)
            for g in range(G):
                hs_ref[g, pl.ds(j, 8, stride=SP), :] = hr[:, g * 128:(g + 1) * 128]
                hs_ref[G + g, pl.ds(j, 8, stride=SP), :] = hi[:, g * 128:(g + 1) * 128]

        state['h'] = (jnp.zeros((8, P), f32), jnp.zeros((8, P), f32))
        tasks = [functools.partial(pass1, j) for j in range(S)] + [carry] + \
                [functools.partial(pass2, j) for j in range(S)]

        per = -(-len(tasks) // nfc)
        lnrows = T // NLN
        acts = []
        for n, (f0, f1) in enumerate(fchunks):
            if first and n % DG == 0:
                cp_f[n // DG][0].wait()
                cp_f[n // DG][1].wait()
            g_ = jax.lax.dot_general(xnb, wg_ref[f0:f1, :], _NT, preferred_element_type=f32)
            u_ = jax.lax.dot_general(xnb, wu_ref[f0:f1, :], _NT, preferred_element_type=f32)
            acts.append((jax.nn.gelu(g_, approximate=True) * u_).astype(bf16))
            for t in tasks[n * per:(n + 1) * per]:
                t()
            if 1 <= n < 1 + NLN:
                k = n - 1
                layernorm(xn_ref, nxt, k * lnrows, (k + 1) * lnrows)

        if first:
            for c in cp_c:
                c.wait()
            cp_d.wait()
            cre = cre_ref[...].astype(f32)
            cim = cim_ref[...].astype(f32)
            cw_ref[:, 0:P] = (2.0 * (cre * cr - cim * ci)).astype(bf16)
            cw_ref[:, P:2 * P] = (-2.0 * (cre * ci + cim * cr)).astype(bf16)

        base = base_ref[cur]
        act = jnp.concatenate(acts, axis=1)
        hs = jnp.concatenate(
            [jnp.concatenate([hs_ref[g, c * SP:c * SP + S, :] for c in range(8)], axis=0).astype(bf16)
             for g in range(2 * G)], axis=1)
        y = jax.lax.dot_general(hs, cw_ref[...], _NT, preferred_element_type=f32)
        ffn = jnp.dot(act, wd_ref[...], preferred_element_type=f32)

        o_ref[...] = base + y + ffn

    pl.when(pl.program_id(0) == 0)(lambda: body(True))
    pl.when(pl.program_id(0) != 0)(lambda: body(False))


@jax.jit
def pallas_parallel_sum__ssm_conv_s5__geglu_ffn__prompt_kernel(
    A_x: jax.Array,
    A_Lambda_re: jax.Array,
    A_Lambda_im: jax.Array,
    A_B_re: jax.Array,
    A_B_im: jax.Array,
    A_C_re: jax.Array,
    A_C_im: jax.Array,
    A_log_dt: jax.Array,
    A_Dskip: jax.Array,
    B_x: jax.Array,
    B_w_gate: jax.Array,
    B_w_up: jax.Array,
    B_w_down: jax.Array,
):
    Bsz, L, D = A_x.shape
    assert Bsz == 1
    P = A_Lambda_re.shape[0]
    F = B_w_gate.shape[1]
    T = 256
    FC = 256
    DG = 2
    NLN = 4
    S = T // 8
    nfc = -(-F // FC)
    nsteps = L // T
    assert L % T == 0 and P % 128 == 0 and nfc >= 1 + NLN and T % (8 * NLN) == 0
    x2 = A_x.reshape(L, D)
    bf16 = jnp.bfloat16

    vec = lambda n: pl.BlockSpec((n,), lambda i: (0,))
    hbm = pl.BlockSpec(memory_space=pl.ANY)
    out = pl.pallas_call(
        functools.partial(_kernel, T=T, P=P, F=F, FC=FC, DG=DG, NLN=NLN),
        grid=(nsteps,),
        in_specs=[
            pl.BlockSpec((T, D), lambda i: (0, 0)),
            pl.BlockSpec((T, D), lambda i: (jnp.minimum(i + 1, nsteps - 1), 0)),
            vec(P), vec(P), vec(P), vec(D),
            hbm, hbm, hbm, hbm, hbm, hbm, hbm,
        ],
        out_specs=pl.BlockSpec((T, D), lambda i: (i, 0)),
        out_shape=jax.ShapeDtypeStruct((L, D), jnp.float32),
        scratch_shapes=[
            pltpu.VMEM((P, D), bf16), pltpu.VMEM((P, D), bf16),
            pltpu.VMEM((D, P), bf16), pltpu.VMEM((D, P), bf16),
            pltpu.VMEM((F, D), bf16), pltpu.VMEM((F, D), bf16), pltpu.VMEM((F, D), bf16),
            pltpu.SemaphoreType.DMA((5 + 2 * nfc,)),
            pltpu.VMEM((D, 2 * P), jnp.bfloat16),
            pltpu.VMEM((8, P), jnp.float32),
            pltpu.VMEM((8, P), jnp.float32),
            pltpu.VMEM((2 * P // 128, 8 * (S + 1), 128), jnp.float32),
            pltpu.VMEM((2 * P // 128, 8 * (S + 1), 128), jnp.float32),
            pltpu.VMEM((2, T, D), bf16),
            pltpu.VMEM((2, T, D), jnp.float32),
        ],
        compiler_params=pltpu.CompilerParams(
            dimension_semantics=("arbitrary",),
            vmem_limit_bytes=100 * 1024 * 1024,
        ),
    )(x2, x2, A_Lambda_re, A_Lambda_im, A_log_dt, A_Dskip,
      A_B_re, A_B_im, A_C_re, A_C_im, B_w_gate.T, B_w_up.T, B_w_down)
    return out.reshape(Bsz, L, D)
```
